```python
import os as _os
_os.environ.setdefault("JAX_PLATFORMS", "cpu")
import jax
import jax.numpy as jnp

def _softmax(x, axis=-1):
    return jax.nn.softmax(x, axis=axis)
def _gelu(x):
    return jax.nn.gelu(x, approximate=True)
def _silu(x):
    return jax.nn.silu(x)
def _sigmoid(x):
    return jax.nn.sigmoid(x)
def _layernorm(x, axis=-1, eps=1e-5):
    m = jnp.mean(x, axis=axis, keepdims=True)
    v = jnp.var(x, axis=axis, keepdims=True)
    return (x - m) / jnp.sqrt(v + eps)
def _scatter_add(tgt, idx, src, axis=0):
    return tgt.at[idx].add(src)
def _segment_sum(src, seg, n):
    return jax.ops.segment_sum(src, seg, n)
class _Rng:
    def __init__(self, key):
        self._k = key
    def _next(self):
        self._k, sub = jax.random.split(self._k)
        return sub
    def normal(self, shape):
        return jax.random.normal(self._next(), shape, dtype=jnp.bfloat16)
    def randint(self, lo, hi, shape):
        return jax.random.randint(self._next(), shape, lo, hi, dtype=jnp.int32)
    def uniform(self, shape, lo=0.0, hi=1.0):
        return jax.random.uniform(self._next(), shape, jnp.bfloat16, lo, hi)
    def permutation(self, n):
        return jax.random.permutation(self._next(), n)


kernel_name = 'sequential_preLN__linear_kernel_hedgehog__geglu_ffn__prompt'

def setup_inputs():
    _rng = _Rng(jax.random.key(int.from_bytes(__import__("os").urandom(4), "little")))
    _w = (lambda a: (lambda t: t.astype(jnp.bfloat16) if jnp.issubdtype(t.dtype, jnp.floating) else t)(jnp.asarray(a)))
    def _A_setup():
        B, S, D, H = 1, 2048, 640, 32
        Dh = D // H
        return {
            "x": _w((lambda *s: _rng.normal(s) * 0.05)(B, S, D)),
            "wqkv": _w((lambda *s: _rng.normal(s) * 0.2)(D, 3 * D)),
            "w_phi": _w((lambda *s: _rng.normal(s) * 0.2)(H, Dh, Dh) * (Dh ** -0.5)),
            "wo": _w((lambda *s: _rng.normal(s) * 0.05)(D, D)),
        }
    _A_in = _A_setup()

    def _B_setup():
        B, S, D, F = 1, 2048, 640, 1536
        return {
            "x": _w((lambda *s: _rng.normal(s) * 0.05)(B, S, D)),
            "w_gate": _w((lambda *s: _rng.normal(s) * 0.05)(D, F)),
            "w_up": _w((lambda *s: _rng.normal(s) * 0.05)(D, F)),
            "w_down": _w((lambda *s: _rng.normal(s) * 0.05)(F, D)),
        }
    _B_in = _B_setup()

    return {
        "A_x": _A_in["x"],
        "A_wqkv": _A_in["wqkv"],
        "A_w_phi": _A_in["w_phi"],
        "A_wo": _A_in["wo"],
        "B_x": _B_in["x"],
        "B_w_gate": _B_in["w_gate"],
        "B_w_up": _B_in["w_up"],
        "B_w_down": _B_in["w_down"],
    }

def reference(A_x, A_wqkv, A_w_phi, A_wo, B_x, B_w_gate, B_w_up, B_w_down):
    def _A_ref(x, wqkv, w_phi, wo):
        B, S, D = x.shape
        H = 32; Dh = D // H
        qkv = (lambda x, *d: x.transpose(*d))((x @ wqkv).reshape(B, S, 3, H, Dh), 2, 0, 3, 1, 4)
        q, k, v = qkv[0], qkv[1], qkv[2]
        pq = jnp.einsum("bhsd,hdf->bhsf", q, w_phi)
        pk = jnp.einsum("bhsd,hdf->bhsf", k, w_phi)
        phi_q = jnp.concatenate([_softmax(pq, axis=-1), _softmax(-pq, axis=-1)], axis=-1)
        phi_k = jnp.concatenate([_softmax(pk, axis=-1), _softmax(-pk, axis=-1)], axis=-1)
        kv = jnp.einsum("bhsf,bhsd->bhfd", phi_k, v)
        z  = jnp.einsum("bhsf->bhf", phi_k)
        num = jnp.einsum("bhqf,bhfd->bhqd", phi_q, kv)
        den = jnp.einsum("bhqf,bhf->bhq", phi_q, z)[..., None] + 1e-6
        o = num / den
        return (lambda x, *d: x.transpose(*d))(o, 0, 2, 1, 3).reshape(B, S, D) @ wo

    def _B_ref(x, w_gate, w_up, w_down):
        return (_gelu(x @ w_gate) * (x @ w_up)) @ w_down

    x = A_x
    h = x + _A_ref(_layernorm(x, axis=-1), A_wqkv, A_w_phi, A_wo)
    h2 = h + _B_ref(_layernorm(h, axis=-1), B_w_gate, B_w_up, B_w_down)
    return h2
```

```python
import jax
import jax.numpy as jnp
from jax import lax
import jax.experimental.pallas as pl
import jax.experimental.pallas.tpu as pltpu
import contextlib
PROF = False
def scope(n):
    return jax.named_scope(n) if PROF else contextlib.nullcontext()

S, D, H, DH, F = 2048, 640, 32, 20, 1536
NP = H // 2
PR = 2 * DH
EXT = PR + 8
QR = 2 * PR
LOG2E = 1.4426950408889634
T1 = 512
T2 = 256
FS = 5
LATE = (.5, .5, 1, 2, 2)
PRIO = 0
XW = 2
LP = 3
WW = 2
FP = 3
NH = 2
FC = 512
PV = 160
PQ = 640
LNPOS = 0
ORDER = 'faffafa'
PM = 640
FLAGS = None
VMEM_LIMIT = 100 * 1024 * 1024

f32, bf16 = jnp.float32, jnp.bfloat16
NT = (((1,), (1,)), ((), ()))


def _layernorm(x):
    m = jnp.mean(x, axis=-1, keepdims=True)
    c = x - m
    v = jnp.mean(c * c, axis=-1, keepdims=True)
    return c * lax.rsqrt(v + 1e-5)


def _allreduce(op, slabs):
    r = slabs[0]
    for s in slabs[1:]:
        r = op(r, s)
    r = op(r, pltpu.roll(r, 4, 0))
    return op(r, pltpu.roll(r, 2, 0))


def _features(p):
    sl = [p[8 * i:8 * (i + 1)] for i in range(PR // 8)]
    mx = _allreduce(jnp.maximum, sl)
    mn = _allreduce(jnp.minimum, sl)
    ep = [jnp.exp2(s - mx) for s in sl]
    en = [jnp.exp2(mn - s) for s in sl]
    rp = 1.0 / _allreduce(jnp.add, ep)
    rn = 1.0 / _allreduce(jnp.add, en)
    return jnp.concatenate([a * rp for a in ep] + [b * rn for b in en], axis=0).astype(bf16)


def _normalize(nd):
    inv = 1.0 / (nd[PR:EXT] + 1e-6)
    swapped = pltpu.roll(inv, 4, 0)
    low = lax.broadcasted_iota(jnp.int32, inv.shape, 0) < 4
    i0, i1 = jnp.where(low, inv, swapped), jnp.where(low, swapped, inv)
    return nd[:PR] * jnp.concatenate([i0, i0, inv, i1, i1], axis=0)


def _quad_window(q):
    lo, hi = (QR * q) // 128, (QR * q + QR - 1) // 128 + 1
    return 128 * lo, 128 * hi


def _kernel(x_hbm, wqkv_hbm, wphi_hbm, wo_hbm, wg_hbm, wu_hbm, wd_hbm, o_hbm,
            x_v, xn_v, wqkv_v, wphi_v, wo_v, wg_v, wu_v, wd_v, s_v, bd_v, wkv_t, wq_t,
            acc, lhs2, h_v, hn_v, o_v, sem_x, sem_w, sem_o):
    n1, n2 = S // T1, S // T2

    XCH = [(0, T1 // 2), (T1 // 2, T1 // 2), (T1, S - T1)]

    def x_copy(i):
        rows = pl.ds(*XCH[i])
        return pltpu.make_async_copy(x_hbm.at[rows], x_v.at[rows], sem_x.at[i])

    def qkv_copy(j):
        return pltpu.make_async_copy(wqkv_hbm.at[:, pl.ds(j * D, D)], wqkv_v.at[j], sem_w.at[j])

    c_phi = pltpu.make_async_copy(wphi_hbm, wphi_v, sem_w.at[3])
    c_wq = qkv_copy(0)
    c_wo = pltpu.make_async_copy(wo_hbm, wo_v, sem_w.at[4])
    c_wg = pltpu.make_async_copy(wg_hbm, wg_v, sem_w.at[5])
    c_wu = pltpu.make_async_copy(wu_hbm, wu_v, sem_w.at[6])
    c_wd = pltpu.make_async_copy(wd_hbm, wd_v, sem_w.at[7])

    c_phi.start()
    qkv_copy(1).start()
    x_copy(0).start()
    x_copy(1).start()
    qkv_copy(2).start()
    for i in range(2, len(XCH)):
        x_copy(i).start()
    def start_weights(stage):
        for c, st in zip((c_wq, c_wo, c_wg, c_wu, c_wd), LATE):
            if st == stage:
                c.start(priority=PRIO)

    start_weights(0)

    s_v[...] = jnp.zeros(s_v.shape, f32)
    rr = lax.broadcasted_iota(jnp.int32, (D, D), 0)
    cc = lax.broadcasted_iota(jnp.int32, (D, D), 1)
    perm = jnp.where(cc == (rr & (H - 1)) * DH + (rr >> 5), 1.0, 0.0).astype(bf16)
    rr = lax.broadcasted_iota(jnp.int32, (QR, 32), 0)
    cc = lax.broadcasted_iota(jnp.int32, (QR, 32), 1)
    rep = jnp.where(cc == (jnp.where(rr >= PR, rr - PR, rr) >> 1), 1.0, 0.0).astype(bf16)
    with scope('WPHI'):
        c_phi.wait()
    for d in range(DH):
        s_v[0:DH, d * H:(d + 1) * H] = wphi_v[d].astype(f32)
    a = jnp.dot(s_v[...].astype(bf16), perm, preferred_element_type=f32)
    a = jnp.dot(rep, a.astype(bf16), preferred_element_type=f32)
    for q in range(NP // 2):
        lo, hi = _quad_window(q)
        r = lax.broadcasted_iota(jnp.int32, (QR, hi - lo), 0)
        c = lax.broadcasted_iota(jnp.int32, (QR, hi - lo), 1) + lo
        first = (4 * q + jnp.where(r >= PR, 2, 0) + (r & 1)) * DH
        bd_v[q, :, 0:hi - lo] = jnp.where((c >= first) & (c < first + DH), a[:, lo:hi], 0.0).astype(bf16)

    def fold(j, dst, quads):
        for q in quads:
            lo, hi = _quad_window(q)
            w = lax.dot_general(bd_v[q, :, 0:hi - lo], wqkv_v[j, :, lo:hi], NT, preferred_element_type=f32)
            dst[QR * q:QR * (q + 1), :] = (w * LOG2E).astype(bf16)

    def norm_rows(start, size):
        rows = pl.ds(start, size)
        xn_v[rows, :] = _layernorm(x_v[rows, :].astype(f32)).astype(bf16)

    def k_proj(start, size, lo=0, hi=D):
        return lax.dot_general(wkv_t[lo:hi, :], xn_v[pl.ds(start, size), :], NT, preferred_element_type=f32)

    def kv_update(i, p, hooks):
        xn = xn_v[pl.ds(i * T1, T1), :]
        ones = jnp.ones((8, T1), f32)
        phis = [_features(p[PR * j:PR * (j + 1)]) for j in range(NP)]
        for m in range(D // PV):
            hooks.get(m, lambda: None)()
            v = lax.dot_general(wkv_t[D + PV * m:D + PV * (m + 1), :], xn, NT, preferred_element_type=f32)
            for j in range(PV // PR):
                ve = jnp.concatenate([v[PR * j:PR * (j + 1)], ones], axis=0).astype(bf16)
                jj = m * (PV // PR) + j
                kv = lax.dot_general(ve, phis[jj], NT, preferred_element_type=f32)
                acc[jj] = kv if i == 0 else acc[jj] + kv

    def wait_weights():
        c_wq.wait()
        c_wo.wait()
        c_wg.wait()
        c_wu.wait()
        c_wd.wait()

    th = T1 // 2
    with scope('Wk'):
        qkv_copy(1).wait()
    fold(1, wkv_t, range(0, FS))
    x_copy(0).wait()
    fold(1, wkv_t, range(FS, NP // 2))
    norm_rows(0, th)
    x_copy(1).wait()
    p_a = k_proj(0, th)
    norm_rows(th, th)
    p_b0 = k_proj(th, th, 0, D // 2)
    qkv_copy(2).wait()
    p_b1 = k_proj(th, th, D // 2, D)
    wkv_t[D:2 * D, :] = wqkv_v[2].T
    kv_update(0, jnp.concatenate([p_a, jnp.concatenate([p_b0, p_b1], axis=0)], axis=1),
              {XW: lambda: (x_copy(2).wait(), start_weights(0.5)), LP: lambda: norm_rows(T1, T1)})
    for i in range(1, n1):
        start_weights(i)
        if i + 1 < n1:
            hooks = {LP: lambda: norm_rows((i + 1) * T1, T1)}
        else:
            hooks = {WW: wait_weights, FP: lambda: fold(0, wq_t, range(NP // 2))}
        with scope(f'T{i}'):
            kv_update(i, k_proj(i * T1, T1), hooks)

    r = lax.broadcasted_iota(jnp.int32, (EXT, 2 * PR), 0)
    hc = lax.broadcasted_iota(jnp.int32, (EXT, 2 * PR), 1) & 1
    hr = jnp.where(((r >= DH) & (r < PR)) | (r >= PR + 4), 1, 0)
    for j in range(NP):
        lhs2[j] = jnp.where(hr == hc, acc[j], 0.0).astype(bf16)

    def tile_rows(i):
        return pl.ds(i * T2 if isinstance(i, int) else pl.multiple_of(i * T2, T2), T2)

    def o_copy(i):
        return pltpu.make_async_copy(o_v.at[tile_rows(i)], o_hbm.at[tile_rows(i)], sem_o.at[i])

    def attention(i, slot):
        xn = xn_v[tile_rows(i), :]
        ps = []
        for m in range(D // PQ):
            ps.append(lax.dot_general(wq_t[PQ * m:PQ * (m + 1), :], xn, NT, preferred_element_type=f32))
        phis = [_features(p[PR * j:PR * (j + 1)]) for p in ps for j in range(PQ // PR)]
        yield
        ot = [_normalize(jnp.dot(lhs2[j], phis[j], preferred_element_type=f32)) for j in range(NP)]
        o = jnp.concatenate(ot, axis=0).astype(bf16).T
        yield
        h = x_v[tile_rows(i), :].astype(f32) + jnp.dot(o, wo_v[...], preferred_element_type=f32)
        h_v[slot] = h
        hn_v[slot] = _layernorm(h).astype(bf16)
        yield

    def ffn(i, slot):
        hn = hn_v[slot]
        y = h_v[slot]
        for c in range(F // FC):
            cols = slice(c * FC, (c + 1) * FC)
            gt = jnp.dot(hn, wg_v[:, cols], preferred_element_type=f32)
            up = jnp.dot(hn, wu_v[:, cols], preferred_element_type=f32)
            inner = gt * (0.7978845608028654 + 0.7978845608028654 * 0.044715 * (gt * gt))
            hg = (0.5 * gt) * up
            a = (hg + hg * jnp.tanh(inner)).astype(bf16)
            yield
            y = y + jnp.dot(a, wd_v[cols, :], preferred_element_type=f32)
            yield
        o_v[tile_rows(i), :] = y.astype(bf16)
        o_copy(i).start()

    def run(order, gens):
        for g in order:
            next(gens[g], None)
        for g in gens.values():
            for _ in g:
                pass

    with scope('MID'):
        run("", {"a": attention(0, 0)})

    def phase2(i, carry):
        run(ORDER, {"a": attention(i + 1, (i + 1) & 1), "f": ffn(i, i & 1)})
        return carry

    with scope('P2'):
        lax.fori_loop(0, n2 - 1, phase2, 0)
    with scope('EPI'):
        run("", {"f": ffn(n2 - 1, (n2 - 1) & 1)})
    with scope('TAIL'):
        for i in range(n2):
            o_copy(i).wait()


@jax.jit
def pallas_sequential_preLN__linear_kernel_hedgehog__geglu_ffn__prompt_kernel(
    A_x: jax.Array,
    A_wqkv: jax.Array,
    A_w_phi: jax.Array,
    A_wo: jax.Array,
    B_x: jax.Array,
    B_w_gate: jax.Array,
    B_w_up: jax.Array,
    B_w_down: jax.Array,
):
    del B_x
    any_spec = pl.BlockSpec(memory_space=pl.ANY)
    out = pl.pallas_call(
        _kernel,
        in_specs=[any_spec] * 7,
        out_specs=any_spec,
        out_shape=jax.ShapeDtypeStruct((S, D), bf16),
        scratch_shapes=[
            pltpu.VMEM((S, D), bf16),
            pltpu.VMEM((S, D), bf16),
            pltpu.VMEM((3, D, D), bf16),
            pltpu.VMEM((DH, DH, H), bf16),
            pltpu.VMEM((D, D), bf16),
            pltpu.VMEM((D, F), bf16),
            pltpu.VMEM((D, F), bf16),
            pltpu.VMEM((F, D), bf16),
            pltpu.VMEM((32, D), f32),
            pltpu.VMEM((NP // 2, QR, 256), bf16),
            pltpu.VMEM((2 * D, D), bf16),
            pltpu.VMEM((D, D), bf16),
            pltpu.VMEM((NP, EXT, 2 * PR), f32),
            pltpu.VMEM((NP, EXT, 2 * PR), bf16),
            pltpu.VMEM((2, T2, D), f32),
            pltpu.VMEM((2, T2, D), bf16),
            pltpu.VMEM((S, D), bf16),
            pltpu.SemaphoreType.DMA((3,)),
            pltpu.SemaphoreType.DMA((8,)),
            pltpu.SemaphoreType.DMA((S // T2,)),
        ],
        compiler_params=pltpu.CompilerParams(vmem_limit_bytes=VMEM_LIMIT, flags=FLAGS),
    )(A_x.reshape(S, D), A_wqkv, jnp.transpose(A_w_phi, (1, 2, 0)), A_wo, B_w_gate, B_w_up, B_w_down)
    return out.reshape(1, S, D)
```

```python
import jax
import jax.numpy as jnp
from jax import lax
import jax.experimental.pallas as pl
import jax.experimental.pallas.tpu as pltpu

S, D, H, DH, F = 2048, 640, 32, 20, 1536
NP = H // 2
PR = 2 * DH
EXT = PR + 8
QR = 2 * PR
LOG2E = 1.4426950408889634
T1 = 512
T2 = 256
FC = 256
PM = 320
PV = 160
PB = 160
LC = 128
FS = 5
ORDER = "cfaffaffa"
ORDER0 = "zzzcaffaffa"
VMEM_LIMIT = 100 * 1024 * 1024

f32, bf16 = jnp.float32, jnp.bfloat16


def _dot(a, b):
    return jnp.dot(a, b, preferred_element_type=f32)


def _dot_nt(a, b):
    return lax.dot_general(a, b, (((1,), (1,)), ((), ())), preferred_element_type=f32)


def _pack(v):
    return pltpu.bitcast(v.astype(bf16), jnp.int32)


def _unpack(v):
    return pltpu.bitcast(v, bf16)


def _packed(*shape):
    return pltpu.VMEM(shape[:-2] + (shape[-2] // 2, shape[-1]), jnp.int32)


def _rows(start, size):
    if isinstance(start, int):
        return pl.ds(start // 2, size // 2)
    return pl.ds(pl.multiple_of(start // 2, size // 2), size // 2)


def _layernorm(x):
    m = jnp.mean(x, axis=-1, keepdims=True)
    c = x - m
    v = jnp.mean(c * c, axis=-1, keepdims=True)
    return c * lax.rsqrt(v + 1e-5)


def _allreduce(op, slabs):
    r = slabs[0]
    for s in slabs[1:]:
        r = op(r, s)
    r = op(r, pltpu.roll(r, 4, 0))
    return op(r, pltpu.roll(r, 2, 0))


def _features(p):
    sl = [p[8 * i:8 * (i + 1)] for i in range(PR // 8)]
    mx = _allreduce(jnp.maximum, sl)
    mn = _allreduce(jnp.minimum, sl)
    ep = [jnp.exp2(s - mx) for s in sl]
    en = [jnp.exp2(mn - s) for s in sl]
    rp = 1.0 / _allreduce(jnp.add, ep)
    rn = 1.0 / _allreduce(jnp.add, en)
    return jnp.concatenate([a * rp for a in ep] + [b * rn for b in en], axis=0).astype(bf16)


def _normalize(nd):
    inv = 1.0 / (nd[PR:EXT] + 1e-6)
    swapped = pltpu.roll(inv, 4, 0)
    low = lax.broadcasted_iota(jnp.int32, inv.shape, 0) < 4
    i0, i1 = jnp.where(low, inv, swapped), jnp.where(low, swapped, inv)
    return nd[:PR] * jnp.concatenate([i0, i0, inv, i1, i1], axis=0)


def _geglu(gate, up):
    inner = gate * (0.7978845608028654 + 0.7978845608028654 * 0.044715 * (gate * gate))
    half = (0.5 * gate) * up
    return half + half * jnp.tanh(inner)


def _left_factors(a11, a12, a21, a22):
    return [a11 + a22, a21 + a22, a11, a22, a11 + a12, a21 - a11, a12 - a22]


def _right_sums(b11, b12, b21, b22):
    b11, b12, b21, b22 = [b.astype(f32) for b in (b11, b12, b21, b22)]
    return [_pack(s) for s in (b11 + b22, b12 - b22, b21 - b11, b11 + b12, b21 + b22)]


def _strassen(left, sums, b11, b22):
    right = [sums[0], b11, sums[1], sums[2], b22, sums[3], sums[4]]
    m = [_dot(a, b) for a, b in zip(left, right)]
    return m[0] + m[3] - m[4] + m[6], m[2] + m[4], m[1] + m[3], m[0] - m[1] + m[2] + m[5]


def _around(blocks, mid):
    c11, c12, c21, c22 = blocks
    return jnp.concatenate([jnp.concatenate([c11, c21], axis=0), mid, jnp.concatenate([c12, c22], axis=0)], axis=1)


def _quad_window(q):
    return 128 * ((QR * q) // 128), 128 * ((QR * q + QR - 1) // 128 + 1)


def _kernel(x_hbm, wqkv_hbm, wphi_hbm, wo_hbm, wg_hbm, wu_hbm, wd_hbm, o_hbm,
            x_v, o_v, wqkv_v, wphi_v, wo_v, wg_v, wu_v, wd_v, s_v, bd_v,
            xn_v, wk_t, wv_t, wq_t, acc, kv_v, h_v, hn_v, hn_next, so_v, sg_v, sd_v,
            sem_x, sem_w, sem_o):
    n1, n2, th, t2 = S // T1, S // T2, T1 // 2, T2 // 2

    def row_copies(src, dst, spans, sem):
        return [pltpu.make_async_copy(src.at[pl.ds(*s)], dst.at[pl.ds(*s)], sem.at[i]) for i, s in enumerate(spans)]

    c_x = row_copies(x_hbm, x_v, [(0, th), (th, th), (T1, S - T1)], sem_x)
    c_o = row_copies(o_v, o_hbm, [(0, S - T2), (S - T2, T2)], sem_o)
    c_wq, c_wk, c_wv = [pltpu.make_async_copy(wqkv_hbm.at[:, pl.ds(j * D, D)], wqkv_v.at[j], sem_w.at[j])
                        for j in range(3)]
    c_phi = pltpu.make_async_copy(wphi_hbm, wphi_v, sem_w.at[3])
    c_wo = pltpu.make_async_copy(wo_hbm, wo_v, sem_w.at[4])
    c_wg = pltpu.make_async_copy(wg_hbm, wg_v, sem_w.at[5])
    c_wu = pltpu.make_async_copy(wu_hbm, wu_v, sem_w.at[6])
    c_wd = pltpu.make_async_copy(wd_hbm, wd_v, sem_w.at[7])

    c_phi.start()
    c_wk.start()

    s_v[...] = jnp.zeros(s_v.shape, f32)
    rr = lax.broadcasted_iota(jnp.int32, (D, D), 0)
    cc = lax.broadcasted_iota(jnp.int32, (D, D), 1)
    perm = jnp.where(cc == (rr & (H - 1)) * DH + (rr >> 5), 1.0, 0.0).astype(bf16)
    rr = lax.broadcasted_iota(jnp.int32, (QR, 32), 0)
    cc = lax.broadcasted_iota(jnp.int32, (QR, 32), 1)
    rep = jnp.where(cc == (jnp.where(rr >= PR, rr - PR, rr) >> 1), 1.0, 0.0).astype(bf16)
    c_phi.wait()
    c_x[0].start()
    c_x[1].start()
    for d in range(DH):
        s_v[0:DH, d * H:(d + 1) * H] = wphi_v[d].astype(f32)
    a = _dot(s_v[...].astype(bf16), perm)
    a = _dot(rep, a.astype(bf16))
    for q in range(NP // 2):
        lo, hi = _quad_window(q)
        r = lax.broadcasted_iota(jnp.int32, (QR, hi - lo), 0)
        c = lax.broadcasted_iota(jnp.int32, (QR, hi - lo), 1) + lo
        first = (4 * q + jnp.where(r >= PR, 2, 0) + (r & 1)) * DH
        bd_v[q, :, 0:hi - lo] = _pack(jnp.where((c >= first) & (c < first + DH), a[:, lo:hi], 0.0))

    def fold(dst, j, quads):
        for q in quads:
            lo, hi = _quad_window(q)
            w = _dot_nt(_unpack(bd_v[q, :, 0:hi - lo]), wqkv_v[j, :, lo:hi])
            dst[_rows(QR * q, QR), :] = _pack(w * LOG2E)

    def norm_rows(start, size):
        for r in range(start, start + size, LC):
            xn_v[_rows(r, LC), :] = _pack(_layernorm(x_v[pl.ds(r, LC), :].astype(f32)))

    def project(w_t, lo, m, start, size):
        p = _dot_nt(_unpack(w_t[_rows(lo, m), :]), _unpack(xn_v[_rows(start, size), :]))
        return [p[r:r + PR] for r in range(0, m, PR)]

    def project_all(w_t, start, size):
        return [p for lo in range(0, D, PM) for p in project(w_t, lo, PM, start, size)]

    def kv_update(start, pk, before_last):
        phis = [_features(p) for p in pk]
        for lo in range(0, D, PV):
            if lo == D - PV:
                before_last()
            for k, v in enumerate(project(wv_t, lo, PV, start, T1)):
                j = lo // PR + k
                ve = jnp.concatenate([v, jnp.ones((8, T1), f32)], axis=0).astype(bf16)
                kv = _dot_nt(ve, phis[j])
                acc[j] = kv if start == 0 else acc[j] + kv

    c_wk.wait()
    c_wv.start()
    fold(wk_t, 1, range(0, FS))
    c_x[0].wait()
    c_x[2].start()
    fold(wk_t, 1, range(FS, NP // 2))
    norm_rows(0, th)
    c_x[1].wait()
    p_a = project(wk_t, 0, D, 0, th)
    norm_rows(th, th)
    p_b = project(wk_t, 0, PB, th, th)
    c_wv.wait()
    p_b += project(wk_t, PB, D - PB, th, th)
    wv_t[...] = _pack(wqkv_v[2].T)

    def second_tile():
        c_x[2].wait()
        c_wq.start(priority=1)
        c_wo.start(priority=1)
        norm_rows(T1, T1)

    kv_update(0, [jnp.concatenate(ab, axis=1) for ab in zip(p_a, p_b)], second_tile)
    for i, copies in enumerate([(c_wg,), (c_wu, c_wd), ()], start=1):
        for c in copies:
            c.start(priority=1)
        kv_update(i * T1, project_all(wk_t, i * T1, T1),
                  lambda: norm_rows((i + 1) * T1, T1) if i + 1 < n1 else None)

    for c in (c_wq, c_wo, c_wg, c_wu, c_wd):
        c.wait()
    fold(wq_t, 0, range(NP // 2))
    r = lax.broadcasted_iota(jnp.int32, (EXT, 2 * PR), 0)
    col_head = lax.broadcasted_iota(jnp.int32, (EXT, 2 * PR), 1) & 1
    row_head = jnp.where(((r >= DH) & (r < PR)) | (r >= PR + 4), 1, 0)
    for j in range(NP):
        kv_v[j] = _pack(jnp.where(row_head == col_head, acc[j], 0.0))

    def tile_rows(i):
        return pl.ds(i * T2 if isinstance(i, int) else pl.multiple_of(i * T2, T2), T2)

    def attention(i, slot, first=False):
        phis = [_features(p) for p in project_all(wq_t, i * T2, T2)]
        yield
        ot = jnp.concatenate([_normalize(_dot(_unpack(kv_v[j]), phis[j])) for j in range(NP)], axis=0)
        a11, a12, a21, a22 = ot[:256, :t2], ot[384:, :t2], ot[:256, t2:], ot[384:, t2:]
        left = [v.astype(bf16).T for v in _left_factors(a11, a12, a21, a22)]
        a12, a21, rest = a12.astype(bf16).T, a21.astype(bf16).T, ot[256:384].astype(bf16).T
        yield
        if first:
            for k, s in enumerate(_right_sums(wo_v[:256, :256], wo_v[:256, 384:], wo_v[384:, :256], wo_v[384:, 384:])):
                so_v[k] = s
        blocks = _strassen(left, [_unpack(so_v[k]) for k in range(5)], wo_v[:256, :256], wo_v[384:, 384:])
        mid = (_dot(jnp.concatenate([left[2], a21], axis=0), wo_v[:256, 256:384])
               + _dot(jnp.concatenate([a12, left[3]], axis=0), wo_v[384:, 256:384]))
        h = x_v[tile_rows(i), :].astype(f32) + (_around(blocks, mid) + _dot(rest, wo_v[256:384, :]))
        h_v[slot] = h
        hn = _layernorm(h)
        left = _left_factors(hn[:t2, :256], hn[:t2, 384:], hn[t2:, :256], hn[t2:, 384:])
        hn_next[...] = _pack(jnp.concatenate(left + [hn[:t2, 256:384], hn[t2:, 256:384]], axis=1))
        yield

    def advance():
        hn_v[...] = hn_next[...]
        yield

    def gate_up_block(row, c, half):
        rows, cols = pl.ds(row, 256), pl.ds(c * FC + half * (FC // 2), FC // 2)
        return jnp.concatenate([wg_v[rows, cols], wu_v[rows, cols]], axis=1)

    def activations(c, first):
        cols = slice(c * FC, (c + 1) * FC)
        if first:
            for k, s in enumerate(_right_sums(gate_up_block(0, c, 0), gate_up_block(0, c, 1),
                                              gate_up_block(384, c, 0), gate_up_block(384, c, 1))):
                sg_v[k, :, cols] = s
        c11, c12, c21, c22 = _strassen(
            [_unpack(hn_v[:, 256 * k:256 * (k + 1)]) for k in range(7)],
            [_unpack(sg_v[k, :, cols]) for k in range(5)], gate_up_block(0, c, 0), gate_up_block(384, c, 1))
        rest = jnp.concatenate([_unpack(hn_v[:, 1792:1920]), _unpack(hn_v[:, 1920:2048])], axis=0)

        def assemble(part, w_v):
            top = jnp.concatenate([c11[:, part], c12[:, part]], axis=1)
            bot = jnp.concatenate([c21[:, part], c22[:, part]], axis=1)
            return jnp.concatenate([top, bot], axis=0) + _dot(rest, w_v[256:384, cols])

        return _geglu(assemble(slice(0, FC // 2), wg_v), assemble(slice(FC // 2, FC), wu_v))

    def ffn(i, slot, first=False):
        acts, k = [], F // 2
        for c in range(F // FC):
            acts.append(activations(c, first))
            if first:
                lo, hi = c * FC // 2, (c + 1) * FC // 2
                for j, s in enumerate(_right_sums(wd_v[lo:hi, :256], wd_v[lo:hi, 384:],
                                                  wd_v[k + lo:k + hi, :256], wd_v[k + lo:k + hi, 384:])):
                    sd_v[j, _rows(lo, hi - lo)] = s
            yield
        act = jnp.concatenate(acts, axis=1)
        left = [v.astype(bf16) for v in _left_factors(act[:t2, :k], act[:t2, k:], act[t2:, :k], act[t2:, k:])]
        blocks = _strassen(left, [_unpack(sd_v[j]) for j in range(5)], wd_v[:k, :256], wd_v[k:, 384:])
        y = _around(blocks, _dot(act.astype(bf16), wd_v[:, 256:384]))
        o_v[tile_rows(i), :] = (h_v[slot] + y).astype(bf16)

    def run(order, **stages):
        for name in order:
            next(stages[name], None)
        for stage in stages.values():
            for _ in stage:
                pass

    def step(i, carry):
        run(ORDER, c=advance(), a=attention(i + 1, (i + 1) & 1), f=ffn(i, i & 1))
        return carry

    run(ORDER0, z=attention(0, 0, True), c=advance(), a=attention(1, 1), f=ffn(0, 0, True))
    lax.fori_loop(1, n2 - 1, step, 0)
    c_o[0].start()
    run("cf", c=advance(), f=ffn(n2 - 1, (n2 - 1) & 1))
    c_o[1].start()
    c_o[0].wait()
    c_o[1].wait()


@jax.jit
def pallas_sequential_preLN__linear_kernel_hedgehog__geglu_ffn__prompt_kernel(
    A_x: jax.Array,
    A_wqkv: jax.Array,
    A_w_phi: jax.Array,
    A_wo: jax.Array,
    B_x: jax.Array,
    B_w_gate: jax.Array,
    B_w_up: jax.Array,
    B_w_down: jax.Array,
):
    del B_x
    any_spec = pl.BlockSpec(memory_space=pl.ANY)
    out = pl.pallas_call(
        _kernel,
        in_specs=[any_spec] * 7,
        out_specs=any_spec,
        out_shape=jax.ShapeDtypeStruct((S, D), bf16),
        scratch_shapes=[
            pltpu.VMEM((S, D), bf16),
            pltpu.VMEM((S, D), bf16),
            pltpu.VMEM((3, D, D), bf16),
            pltpu.VMEM((DH, DH, H), bf16),
            pltpu.VMEM((D, D), bf16),
            pltpu.VMEM((D, F), bf16),
            pltpu.VMEM((D, F), bf16),
            pltpu.VMEM((F, D), bf16),
            pltpu.VMEM((32, D), f32),
            _packed(NP // 2, QR, 256),
            _packed(S, D),
            _packed(D, D),
            _packed(D, D),
            _packed(D, D),
            pltpu.VMEM((NP, EXT, 2 * PR), f32),
            _packed(NP, EXT, 2 * PR),
            pltpu.VMEM((2, T2, D), f32),
            _packed(T2 // 2, 2048),
            _packed(T2 // 2, 2048),
            _packed(5, 256, 256),
            _packed(5, 256, F),
            _packed(5, F // 2, 256),
            pltpu.SemaphoreType.DMA((3,)),
            pltpu.SemaphoreType.DMA((8,)),
            pltpu.SemaphoreType.DMA((2,)),
        ],
        compiler_params=pltpu.CompilerParams(vmem_limit_bytes=VMEM_LIMIT),
    )(A_x.reshape(S, D), A_wqkv, jnp.transpose(A_w_phi, (1, 2, 0)), A_wo, B_w_gate, B_w_up, B_w_down)
    return out.reshape(1, S, D)
```
